```python
import os as _os
_os.environ.setdefault("JAX_PLATFORMS", "cpu")
import jax
import jax.numpy as jnp

def _softmax(x, axis=-1):
    return jax.nn.softmax(x, axis=axis)
def _gelu(x):
    return jax.nn.gelu(x, approximate=True)
def _silu(x):
    return jax.nn.silu(x)
def _sigmoid(x):
    return jax.nn.sigmoid(x)
def _layernorm(x, axis=-1, eps=1e-5):
    m = jnp.mean(x, axis=axis, keepdims=True)
    v = jnp.var(x, axis=axis, keepdims=True)
    return (x - m) / jnp.sqrt(v + eps)
def _scatter_add(tgt, idx, src, axis=0):
    return tgt.at[idx].add(src)
def _segment_sum(src, seg, n):
    return jax.ops.segment_sum(src, seg, n)
class _Rng:
    def __init__(self, key):
        self._k = key
    def _next(self):
        self._k, sub = jax.random.split(self._k)
        return sub
    def normal(self, shape):
        return jax.random.normal(self._next(), shape, dtype=jnp.bfloat16)
    def randint(self, lo, hi, shape):
        return jax.random.randint(self._next(), shape, lo, hi, dtype=jnp.int32)
    def uniform(self, shape, lo=0.0, hi=1.0):
        return jax.random.uniform(self._next(), shape, jnp.bfloat16, lo, hi)
    def permutation(self, n):
        return jax.random.permutation(self._next(), n)


kernel_name = 'interleave_layers__linear_attn_block__mha_block__prompt'

def setup_inputs():
    _rng = _Rng(jax.random.key(int.from_bytes(__import__("os").urandom(4), "little")))
    _w = (lambda a: (lambda t: t.astype(jnp.bfloat16) if jnp.issubdtype(t.dtype, jnp.floating) else t)(jnp.asarray(a)))
    def _A_setup():
        B, S, D = 1, 2048, 640
        return {
            "x": _w((lambda *s: _rng.normal(s) * 0.05)(B, S, D)),
            "wqkv": _w((lambda *s: _rng.normal(s) * 0.1)(D, 3 * D)),
            "wo": _w((lambda *s: _rng.normal(s) * 0.05)(D, D)),
        }
    _A_in = _A_setup()

    def _B_setup():
        B, S, D, H = 1, 2048, 640, 32
        return {
            "x": _w((lambda *s: _rng.normal(s) * 0.05)(B, S, D)),
            "wqkv": _w((lambda *s: _rng.normal(s) * 0.1)(D, 3 * D)),
            "wo": _w((lambda *s: _rng.normal(s) * 0.05)(D, D)),
        }
    _B_in = _B_setup()

    return {
        "A_x": _A_in["x"],
        "A_wqkv": _A_in["wqkv"],
        "A_wo": _A_in["wo"],
        "B_x": _B_in["x"],
        "B_wqkv": _B_in["wqkv"],
        "B_wo": _B_in["wo"],
    }

def reference(A_x, A_wqkv, A_wo, B_x, B_wqkv, B_wo):
    def _A_ref(x, wqkv, wo):
        B, S, D = x.shape
        H = 32; Dh = D // H
        qkv = (lambda x, *d: x.transpose(*d))((x @ wqkv).reshape(B, S, 3, H, Dh), 2, 0, 3, 1, 4)
        q, k, v = qkv[0], qkv[1], qkv[2]
        phi = lambda t: jnp.where(t > 0, t + 1, jnp.exp(t)) + 1e-6
        pq, pk = phi(q), phi(k)
        kv = jnp.einsum("bhsd,bhse->bhde", pk, v)
        z = jnp.einsum("bhsd->bhd", pk)
        num = jnp.einsum("bhqd,bhde->bhqe", pq, kv)
        den = jnp.einsum("bhqd,bhd->bhq", pq, z)[..., None] + 1e-6
        o = num / den
        return (lambda x, *d: x.transpose(*d))(o, 0, 2, 1, 3).reshape(B, S, D) @ wo

    def _B_ref(x, wqkv, wo):
        B, S, D = x.shape
        H = 32
        Dh = D // H
        qkv = (lambda x, *d: x.transpose(*d))((x @ wqkv).reshape(B, S, 3, H, Dh), 2, 0, 3, 1, 4)
        q, k, v = qkv[0], qkv[1], qkv[2]
        scores = jnp.einsum("bhqd,bhkd->bhqk", q, k) * (Dh ** -0.5)
        p = _softmax(scores, axis=-1)
        o = jnp.einsum("bhqk,bhkd->bhqd", p, v)
        return (lambda x, *d: x.transpose(*d))(o, 0, 2, 1, 3).reshape(B, S, D) @ wo

    x = A_x
    x = x + _A_ref(_layernorm(x, axis=-1), A_wqkv, A_wo)
    x = x + _B_ref(_layernorm(x, axis=-1), B_wqkv, B_wo)
    x = x + _A_ref(_layernorm(x, axis=-1), A_wqkv, A_wo)
    x = x + _B_ref(_layernorm(x, axis=-1), B_wqkv, B_wo)
    return x
```

```python
import functools

import jax
import jax.numpy as jnp
import numpy as np
from jax import lax
from jax.experimental import pallas as pl
from jax.experimental.pallas import tpu as pltpu

S = 2048
D = 640
H = 32
DH = D // H
TC = 512
NC = S // TC
NW = 6
LN_EPS = 1e-5
PHI_EPS = 1e-6
QK_SCALE = float(DH ** -0.5 * np.log2(np.e))

OPT = dict(MC=640, CK1=128, CK2=128, unroll_chunks=False, only=None, skew=1, dep=3, order=0, flags=None, vpre=0)

f32 = jnp.float32
bf16 = jnp.bfloat16
u32 = jnp.uint32


def _win_start(w):
    return min(120 * w - 8 * (w % 2), D - 128)


def _pack(x):
    return pltpu.bitcast(x.astype(bf16), u32)


def _unpack(x):
    return pltpu.bitcast(x, bf16)


def _dot(a, b):
    return lax.dot_general(a, b, (((1,), (0,)), ((), ())), preferred_element_type=f32)


def _dot_nt(a, b):
    return lax.dot_general(a, b, (((1,), (1,)), ((), ())), preferred_element_type=f32)


def _phi(t):
    return jnp.where(t > 0, t + 1.0, jnp.exp(t)) + PHI_EPS


def _head_of(i):
    return (i * 3277) >> 16


def _kernel(x_hbm, wqa_hbm, woa_hbm, wqb_hbm, wob_hbm, out_hbm,
            xraw, wqa, woa, wqb, wob, ostage, sems,
            xT, xnT, wtA, wtB, pkT, gT, mT, zsel, pqo, rden, pqs, qT, kT, kw, vT, sA, sB):
    MC = OPT["MC"]
    CK1 = OPT["CK1"]
    CK2 = OPT["CK2"]

    def chunk_loop(body):
        if OPT["unroll_chunks"]:
            for c in range(NC):
                body(c)
        else:
            def b(c, carry):
                body(c)
                return carry
            lax.fori_loop(0, NC, b, 0)

    def cols(c):
        if isinstance(c, int):
            return pl.ds(c * TC, TC)
        return pl.ds(pl.multiple_of(c * TC, TC), TC)

    def wrows(wt, r0, n):
        return _unpack(wt[pl.ds(r0 // 2, n // 2), :])

    cp_x = [pltpu.make_async_copy(x_hbm.at[pl.ds(c * TC, TC)], xraw.at[pl.ds(c * TC, TC)], sems.at[c])
            for c in range(NC)]
    cp_wqa = pltpu.make_async_copy(wqa_hbm, wqa, sems.at[NC])
    cp_woa = pltpu.make_async_copy(woa_hbm, woa, sems.at[NC + 1])
    cp_wqb = pltpu.make_async_copy(wqb_hbm, wqb, sems.at[NC + 2])
    cp_wob = pltpu.make_async_copy(wob_hbm, wob, sems.at[NC + 3])
    cp_wqa.start()
    for c in range(NC):
        cp_x[c].start()
    cp_woa.start()
    cp_wqb.start()
    cp_wob.start()

    def transpose_w(src, ncol, dst, r0):
        for j in range(ncol // 128):
            dst[pl.ds((r0 + 128 * j) // 2, 64), :] = pltpu.bitcast(src[:, pl.ds(128 * j, 128)].T, u32)

    xnT[pl.ds(D // 2, 8), :] = _pack(jnp.ones((16, S), f32))
    pqo[...] = jnp.zeros(pqo.shape, f32)
    cp_wqa.wait()
    transpose_w(wqa, 3 * D, wtA, 0)
    for c in range(NC):
        cp_x[c].wait()
        xT[:, cols(c)] = xraw[pl.ds(c * TC, TC), :].T.astype(f32)
    cp_woa.wait()
    transpose_w(woa, D, wtA, 3 * D)
    cp_wqb.wait()
    transpose_w(wqb, 3 * D, wtB, 0)
    cp_wob.wait()
    transpose_w(wob, D, wtB, 3 * D)

    def layernorm(x, c):
        mean = jnp.sum(x, axis=0, keepdims=True) * (1.0 / D)
        xc = x - mean
        var = jnp.sum(xc * xc, axis=0, keepdims=True) * (1.0 / D)
        xnT[pl.ds(0, D // 2), cols(c)] = _pack(xc * lax.rsqrt(var + LN_EPS))

    def xn(c):
        return _unpack(xnT[pl.ds(0, D // 2), cols(c)])

    def a1(c):
        layernorm(xT[:, cols(c)], c)
        for r in range(0, D, MC):
            pkT[pl.ds(r // 2, MC // 2), :] = _pack(_phi(_dot(wrows(wtA, D + r, MC), xn(c))))
        for r in range(0, D, MC):
            pqo[pl.ds(r, MC), cols(c)] = _phi(_dot(wrows(wtA, r, MC), xn(c)))
        gT[...] += _dot_nt(_unpack(xnT[:, cols(c)]), _unpack(pkT[...]))

    def a2():
        row = lax.broadcasted_iota(jnp.int32, (H, D), 0)
        col = lax.broadcasted_iota(jnp.int32, (H, D), 1)
        z = jnp.broadcast_to(gT[pl.ds(D, 1), :], (H, D))
        zsel[...] = jnp.where(_head_of(col) == row, z, 0.0)
        for j in range(D // 128):
            h0, h1 = (128 * j) // DH, (128 * j + 127) // DH
            r0 = (DH * h0) // 16 * 16
            r1 = -(-(DH * (h1 + 1)) // 16) * 16
            k0, k1 = r0 // 128 * 128, -(-r1 // 128) * 128
            kv = _dot(wrows(wtA, 2 * D + r0, r1 - r0), gT[pl.ds(0, D), pl.ds(128 * j, 128)].astype(bf16))
            rr = lax.broadcasted_iota(jnp.int32, kv.shape, 0) + r0
            cc = lax.broadcasted_iota(jnp.int32, kv.shape, 1) + 128 * j
            kv = jnp.where(_head_of(rr) == _head_of(cc), kv, 0.0)
            parts = []
            if r0 > k0:
                parts.append(jnp.zeros((r0 - k0, 128), f32))
            parts.append(kv)
            if k1 > r1:
                parts.append(jnp.zeros((k1 - r1, 128), f32))
            kvm = jnp.concatenate(parts, axis=0).astype(bf16)
            wo = _unpack(wtA[pl.ds(3 * D // 2, D // 2), pl.ds(k0, k1 - k0)])
            mT[:, pl.ds(128 * j, 128)] = _pack(_dot(wo, kvm))

    def a3(c):
        den = _dot(zsel[...], pqo[:, cols(c)].astype(bf16))
        rden[...] = 1.0 / (den + PHI_EPS)
        low = lax.broadcasted_iota(jnp.int32, (8, TC), 0) < 4
        for g in range(H // 4):
            b = [jnp.broadcast_to(rden[pl.ds(4 * g + i, 1), :], (8, TC)) for i in range(4)]
            scale = jnp.concatenate(
                [b[0], b[0], jnp.where(low, b[0], b[1]), b[1], b[1],
                 b[2], b[2], jnp.where(low, b[2], b[3]), b[3], b[3]], axis=0)
            pqs[pl.ds(40 * g, 40), :] = _pack(pqo[pl.ds(80 * g, 80), cols(c)] * scale)
        for r in range(0, D, MC):
            xT[pl.ds(r, MC), cols(c)] += _dot(wrows(mT, r, MC), _unpack(pqs[...]))

    def b1(c):
        layernorm(xT[:, cols(c)], c)
        for r in range(0, D, MC):
            kT[pl.ds(r // 2, MC // 2), :] = _pack(_dot(wrows(wtB, D + r, MC), xn(c)))
        for r in range(0, D, MC):
            qT[pl.ds(r // 2, MC // 2), cols(c)] = _pack(_dot(wrows(wtB, r, MC), xn(c)) * QK_SCALE)
        for w in range(NW):
            kt = _unpack(kT[pl.ds(_win_start(w) // 2, 64), :]).T
            rows = pl.ds(c * (TC // 2), TC // 2) if isinstance(c, int) else \
                pl.ds(pl.multiple_of(c * (TC // 2), TC // 2), TC // 2)
            kw[w, rows, :] = pltpu.bitcast(kt, u32)
        for r in range(0, D, MC):
            vT[pl.ds(r, MC), cols(c)] = _dot(wrows(wtB, 2 * D + r, MC), xn(c))

    def head_q(h, c):
        w = (h * 43) >> 8
        rs = jnp.minimum(60 * w - 4 * (w & 1), (D - 128) // 2)
        lo = 10 * h - rs
        q = qT[pl.ds(pl.multiple_of(rs, 8), 64), cols(c)]
        i = lax.broadcasted_iota(jnp.int32, q.shape, 0)
        return w, _unpack(jnp.where((i >= lo) & (i < lo + 10), q, jnp.zeros_like(q)))

    def pass1_chunk(w, q, dst, k, m):
        s = _dot(_unpack(kw[w, pl.ds(k * CK1 // 2, CK1 // 2), :]), q)
        dst[pl.ds(k * CK1, CK1), :] = s
        mm = jnp.max(s.reshape(CK1 // 8, 8, TC), axis=0)
        return mm if m is None else jnp.maximum(m, mm)

    def step(h, c, hn, cn, src, dst, m_cur):
        w, q = head_q(hn, cn)
        off = 4 * (h & 1)
        ws = pl.multiple_of(DH * h - off, 8)
        r = lax.broadcasted_iota(jnp.int32, (24, CK2), 0)
        own = (r >= off) & (r < off + DH)
        n1, n2 = S // CK1, S // CK2
        st = dict(m=None, acc=None, hist=[])

        def p1(k):
            st["m"] = pass1_chunk(w, q, dst, k, st["m"])
            st["hist"].append(st["m"])

        def p2(k):
            mk = m_cur
            d = OPT["dep"]
            if d and len(st["hist"]) >= d:
                mk = jnp.where(always, jnp.broadcast_to(m_cur, (8, TC)), st["hist"][-d])
                mk = jnp.broadcast_to(mk[None], (CK2 // 8, 8, TC)).reshape(CK2, TC)
            p = jnp.exp2(src[pl.ds(k * CK2, CK2), :] - mk).astype(bf16)
            v = jnp.where(own, vT[pl.ds(ws, 24), pl.ds(k * CK2, CK2)], 1.0)
            o = _dot(v, p)
            st["acc"] = o if st["acc"] is None else st["acc"] + o

        always = h >= 0
        ev = [((k + 0.0) / n1, 0, k) for k in range(n1)] + \
             [((k + OPT["skew"] + (0.5 if OPT["order"] == 0 else -0.5)) / n2, 1, k) for k in range(n2)]
        for _, kind, k in sorted(ev):
            (p2 if kind else p1)(k)
        m_new, acc = st["m"], st["acc"]
        den = jnp.where(off == 0, acc[23:24, :], acc[0:1, :])
        r = lax.broadcasted_iota(jnp.int32, (24, TC), 0)
        own = (r >= off) & (r < off + DH)
        pqo[pl.ds(ws, 24), cols(c)] = jnp.where(own, acc * (1.0 / den), pqo[pl.ds(ws, 24), cols(c)])
        return jnp.max(m_new, axis=0, keepdims=True)

    def b2():
        w, q = head_q(jnp.int32(0), 0)
        m = None
        for k in range(S // CK1):
            m = pass1_chunk(w, q, sA, k, m)
        m = jnp.max(m, axis=0, keepdims=True)

        def body(h, m):
            bufs = (sA, sB)
            for c in range(NC):
                hn, cn = (h, c + 1) if c + 1 < NC else (jnp.minimum(h + 1, H - 1), 0)
                m = step(h, c, hn, cn, bufs[c % 2], bufs[(c + 1) % 2], m)
            return m

        lax.fori_loop(0, H, body, m)

    def out_copy(c):
        return pltpu.make_async_copy(ostage.at[pl.ds(c * TC, TC)], out_hbm.at[pl.ds(c * TC, TC)], sems.at[c])

    def b3(it, c):
        for r in range(0, D, MC):
            xT[pl.ds(r, MC), cols(c)] += _dot(wrows(wtB, 3 * D + r, MC), pqo[:, cols(c)].astype(bf16))

        @pl.when(it == 1)
        def _():
            rows = pl.ds(c * TC, TC) if isinstance(c, int) else pl.ds(pl.multiple_of(c * TC, TC), TC)
            ostage[rows, :] = xT[:, cols(c)].astype(bf16).T
            pltpu.make_async_copy(ostage.at[rows], out_hbm.at[rows], sems.at[c]).start()

    def layer_pair(it, carry):
        if OPT["only"] == "b2":
            b2()
            b3(it, 0); b3(it, 1); b3(it, 2); b3(it, 3)
            return carry
        gT[...] = jnp.zeros(gT.shape, f32)
        with jax.named_scope("a1"):
            chunk_loop(a1)
        with jax.named_scope("a2"):
            a2()
        with jax.named_scope("a3b1"):
            chunk_loop(lambda c: (a3(c), b1(c)))
        with jax.named_scope("b2"):
            b2()
        with jax.named_scope("b3"):
            chunk_loop(functools.partial(b3, it))
        return carry

    lax.fori_loop(0, 2, layer_pair, 0)
    for c in range(NC):
        out_copy(c).wait()


def _call(x, wqa, woa, wqb, wob, interpret=False):
    V = pltpu.VMEM
    scratch = [
        V((S, D), bf16), V((D, 3 * D), bf16), V((D, D), bf16), V((D, 3 * D), bf16), V((D, D), bf16),
        V((S, D), bf16), pltpu.SemaphoreType.DMA((NC + 4,)),
        V((D, S), f32),
        V((D // 2 + 8, S), u32),
        V((2 * D, D), u32),
        V((2 * D, D), u32),
        V((D // 2, TC), u32),
        V((D + 16, D), f32),
        V((D // 2, D), u32),
        V((H, D), f32),
        V((D, S), f32),
        V((H, TC), f32),
        V((D // 2, TC), u32),
        V((D // 2, S), u32),
        V((D // 2, TC), u32),
        V((NW, S // 2, 128), u32),
        V((D, S), f32),
        V((S, TC), f32), V((S, TC), f32),
    ]
    return pl.pallas_call(
        lambda *a: _kernel(*a),
        out_shape=jax.ShapeDtypeStruct((S, D), bf16),
        in_specs=[pl.BlockSpec(memory_space=pl.ANY)] * 5,
        out_specs=pl.BlockSpec(memory_space=pl.ANY),
        scratch_shapes=scratch,
        compiler_params=pltpu.CompilerParams(vmem_limit_bytes=100 * 1024 * 1024, flags=OPT["flags"]),
        name="interleave",
        interpret=interpret,
    )(x, wqa, woa, wqb, wob)


@jax.jit
def pallas_interleave_layers__linear_attn_block__mha_block__prompt_kernel(
    A_x: jax.Array,
    A_wqkv: jax.Array,
    A_wo: jax.Array,
    B_x: jax.Array,
    B_wqkv: jax.Array,
    B_wo: jax.Array,
):
    del B_x
    out = _call(A_x.reshape(S, D), A_wqkv, A_wo, B_wqkv, B_wo)
    return out.reshape(A_x.shape)
```

```python
import jax
import jax.numpy as jnp
import numpy as np
from jax import lax
from jax.experimental import pallas as pl
from jax.experimental.pallas import tpu as pltpu

S = 2048
D = 640
H = 32
DH = D // H
TC = 512
NC = S // TC
NW = 6
CK = 128
HU = 4
SKEW = 2
DEP = 5
NT = 4
LN_EPS = 1e-5
PHI_EPS = 1e-6
QK_SCALE = float(DH ** -0.5 * np.log2(np.e))
ONES = np.uint32(0x3F803F80)

f32 = jnp.float32
bf16 = jnp.bfloat16
u32 = jnp.uint32
i32 = jnp.int32


def _pack(x):
    return pltpu.bitcast(x.astype(bf16), u32)


def _unpack(x):
    return pltpu.bitcast(x, bf16)


def _dot(a, b):
    return lax.dot_general(a, b, (((1,), (0,)), ((), ())), preferred_element_type=f32)


def _dot_nt(a, b):
    return lax.dot_general(a, b, (((1,), (1,)), ((), ())), preferred_element_type=f32)


def _phi(t):
    return jnp.where(t > 0, t + 1.0, jnp.exp(t)) + PHI_EPS


def _head_of(i):
    return (i * 3277) >> 16


def _band(j):
    h0, h1 = (128 * j) // DH, (128 * j + 127) // DH
    return (DH * h0) // 16 * 16, -(-(DH * (h1 + 1)) // 16) * 16


def _kernel(x_hbm, wqa_hbm, woa_hbm, wqb_hbm, wob_hbm, out_hbm,
            xraw, wqa, woa, wqb, wob, ostage, sems, osems,
            xT, xnT, wtA, wtB, pkT, gT, gN, mT, zsel, pqo, rden, pqs, qT, kT, kw, vT, sA, sB):
    Q, K, V, O = 0, D, 2 * D, 3 * D

    def cols(c):
        return pl.ds(c * TC, TC)

    def wrows(wt, r0, n=D):
        return _unpack(wt[pl.ds(r0 // 2, n // 2), :])

    def col_copy(src, dst, c0, s):
        return pltpu.make_async_copy(src.at[:, pl.ds(c0, D)], dst.at[:, pl.ds(c0, D)], sems.at[s])

    cp_x = [pltpu.make_async_copy(x_hbm.at[cols(c)], xraw.at[cols(c)], sems.at[c]) for c in range(NC)]
    cp_wk = col_copy(wqa_hbm, wqa, K, NC)
    cp_wq = col_copy(wqa_hbm, wqa, Q, NC + 1)
    cp_wv = col_copy(wqa_hbm, wqa, V, NC + 2)
    cp_woa = pltpu.make_async_copy(woa_hbm, woa, sems.at[NC + 3])
    cp_wqb = pltpu.make_async_copy(wqb_hbm, wqb, sems.at[NC + 4])
    cp_wob = pltpu.make_async_copy(wob_hbm, wob, sems.at[NC + 5])

    def transpose_w(src, c0, dst, r0):
        for j in range(0, D, 128):
            dst[pl.ds((r0 + j) // 2, 64), :] = pltpu.bitcast(src[:, pl.ds(c0 + j, 128)].T, u32)

    def layernorm(x, c):
        mean = jnp.sum(x, axis=0, keepdims=True) * (1.0 / D)
        xc = x - mean
        var = jnp.sum(xc * xc, axis=0, keepdims=True) * (1.0 / D)
        xnT[pl.ds(0, D // 2), cols(c)] = _pack(xc * lax.rsqrt(var + LN_EPS))

    def set_x(x, c):
        xT[:, cols(c)] = x
        layernorm(x, c)

    def load_x(c):
        set_x(xraw[cols(c), :].T.astype(f32), c)

    def proj(wt, r0, c):
        return _dot(wrows(wt, r0), _unpack(xnT[pl.ds(0, D // 2), cols(c)]))

    def scale_heads(c):
        low = lax.broadcasted_iota(i32, (8, TC), 0) < 4
        for g in range(H // 4):
            b = [jnp.broadcast_to(rden[pl.ds(4 * g + i, 1), cols(c)], (8, TC)) for i in range(4)]
            scale = jnp.concatenate(
                [b[0], b[0], jnp.where(low, b[0], b[1]), b[1], b[1],
                 b[2], b[2], jnp.where(low, b[2], b[3]), b[3], b[3]], axis=0)
            pqs[pl.ds(40 * g, 40), cols(c)] = _pack(pqo[pl.ds(80 * g, 80), cols(c)] * scale)

    def a_k(c):
        pkT[:, cols(c)] = _pack(_phi(proj(wtA, K, c)))

    def a_q(c):
        pqo[:, cols(c)] = _phi(proj(wtA, Q, c))

    def a_g(c):
        g = _dot_nt(_unpack(xnT[:, cols(c)]), _unpack(pkT[:, cols(c)]))
        gT[...] = g if c == 0 else gT[...] + g

    def a_kv():
        row = lax.broadcasted_iota(i32, (H, D), 0)
        col = lax.broadcasted_iota(i32, (H, D), 1)
        zsel[...] = jnp.where(_head_of(col) == row, jnp.broadcast_to(gT[pl.ds(D, 1), :], (H, D)), 0.0)
        for j in range(D // 128):
            gN[pl.ds(64 * j, 64), :] = pltpu.bitcast(
                gT[pl.ds(0, D), pl.ds(128 * j, 128)].astype(bf16).T, u32)
        out = []
        for j in range(D // 128):
            r0, r1 = _band(j)
            kv = _dot(wrows(gN, r0, r1 - r0), wqa[:, pl.ds(V + 128 * j, 128)])
            rr = lax.broadcasted_iota(i32, kv.shape, 0) + r0
            cc = lax.broadcasted_iota(i32, kv.shape, 1) + 128 * j
            out.append(jnp.where(_head_of(rr) == _head_of(cc), kv, 0.0).astype(bf16))
        return out

    def a_m(kvs):
        bands = [_band(j) for j in range(D // 128)]
        parts = [_dot(kv, woa[pl.ds(128 * j, 128), :]) for j, kv in enumerate(kvs)]
        for t in range(0, D, 128):
            cuts = sorted({t, t + 128} | {e for b in bands for e in b if t < e < t + 128})
            rows = []
            for lo, hi in zip(cuts[:-1], cuts[1:]):
                terms = [p[lo - r0:hi - r0] for p, (r0, r1) in zip(parts, bands) if r0 <= lo and hi <= r1]
                rows.append(sum(terms[1:], terms[0]))
            mT[:, pl.ds(t, 128)] = pltpu.bitcast(jnp.concatenate(rows, axis=0).astype(bf16).T, u32)

    def a_den(c):
        den = _dot(zsel[...], pqo[:, cols(c)].astype(bf16))
        rden[:, cols(c)] = 1.0 / (den + PHI_EPS)
        scale_heads(c)

    def a_out(c):
        set_x(xT[:, cols(c)] + _dot(wrows(mT, 0), _unpack(pqs[:, cols(c)])), c)

    def b_k(c):
        kT[:, cols(c)] = _pack(proj(wtB, K, c))
        for w in range(NW):
            r0 = min(60 * w - 4 * (w & 1), (D - 128) // 2)
            kt = _unpack(kT[pl.ds(r0, 64), cols(c)]).T
            kw[w, pl.ds(c * TC // 2, TC // 2), :] = pltpu.bitcast(kt, u32)

    def b_q(c):
        qT[:, cols(c)] = _pack(proj(wtB, Q, c) * QK_SCALE)

    def b_v(c):
        vT[:, cols(c)] = proj(wtB, V, c)

    def head_q(h, c):
        w = (h * 43) >> 8
        r0 = jnp.minimum(60 * w - 4 * (w & 1), (D - 128) // 2)
        lo = 10 * h - r0
        q = qT[pl.ds(pl.multiple_of(r0, 8), 64), cols(c)]
        i = lax.broadcasted_iota(i32, q.shape, 0)
        return w, _unpack(jnp.where((i >= lo) & (i < lo + 10), q, jnp.zeros_like(q)))

    def scores(w, q, dst, k, m):
        s = _dot(_unpack(kw[w, pl.ds(k * CK // 2, CK // 2), :]), q)
        dst[pl.ds(k * CK, CK), :] = s
        mm = jnp.max(s.reshape(CK // 8, 8, TC), axis=0)
        return mm if m is None else jnp.maximum(m, mm)

    def step(h, c, nxt, src, dst, m_cur, always, fill=()):
        n = S // CK
        off = 4 * (h & 1)
        ws = pl.multiple_of(DH * h - off, 8)

        def own(width):
            r = lax.broadcasted_iota(i32, (24, width), 0)
            return (r >= off) & (r < off + DH)

        own_ck = own(CK)
        hist, acc = [], []
        if nxt is not None:
            w, q = head_q(*nxt)

        def qk(k):
            hist.append(scores(w, q, dst, k, hist[-1] if hist else None))

        def pv(k):
            m = m_cur
            if len(hist) >= DEP:
                m = jnp.where(always, jnp.broadcast_to(m_cur, (8, TC)), hist[-DEP])
                m = jnp.broadcast_to(m[None], (CK // 8, 8, TC)).reshape(CK, TC)
            p = jnp.exp2(src[pl.ds(k * CK, CK), :] - m).astype(bf16)
            v = jnp.where(own_ck, vT[pl.ds(ws, 24), pl.ds(k * CK, CK)], 1.0)
            o = _dot(v, p)
            acc[:] = [o if not acc else acc[0] + o]

        events = [(k + SKEW + 0.5, k, pv) for k in range(n)] + list(fill)
        if nxt is not None:
            events += [(k + 0.0, k, qk) for k in range(n)]
        for _, k, fn in sorted(events, key=lambda e: e[0]):
            fn(k)
        o = acc[0]
        rden[pl.ds(h, 1), cols(c)] = jnp.where(off == 0, o[23:24, :], o[0:1, :])
        pqo[pl.ds(ws, 24), cols(c)] = jnp.where(own(TC), o, pqo[pl.ds(ws, 24), cols(c)])
        return None if nxt is None else jnp.max(hist[-1], axis=0, keepdims=True)

    def attention(b_out):
        w, q = head_q(jnp.int32(0), 0)
        m = None
        for k in range(S // CK):
            m = scores(w, q, sA, k, m)
        m = jnp.max(m, axis=0, keepdims=True)
        bufs = (sA, sB)

        def group(g, m, last=False):
            one = xnT[pl.ds(D // 2, 8), pl.ds(0, 128)]
            always = jnp.concatenate([one] * (TC // 128), axis=1) == ONES
            for j in range(HU):
                h = g * HU + j
                for c in range(NC):
                    nxt, fill = ((h, c + 1) if c + 1 < NC else (h + 1, 0)), ()
                    if last and j == HU - 1 and c == NC - 1:
                        nxt, fill = None, [(1.0 + 5 * i, i, b_out) for i in range(NC - 1)]
                    m = step(h, c, nxt, bufs[c % 2], bufs[(c + 1) % 2], m, always, fill)
            return m

        g, m = lax.fori_loop(0, H // HU - 1, lambda g, cr: (g + 1, group(g, cr[1])), (jnp.int32(0), m))
        group(g, m, last=True)
        b_out(NC - 1)

    def b_proj(c):
        rden[:, cols(c)] = 1.0 / rden[:, cols(c)]
        scale_heads(c)
        return xT[:, cols(c)] + _dot(wrows(wtB, O), _unpack(pqs[:, cols(c)]))

    def b_out_mid(c):
        set_x(b_proj(c), c)

    def out_copies(c):
        n = NT if c == NC - 1 else 1
        rows = [pl.ds(c * TC + i * (TC // n), TC // n) for i in range(n)]
        return [pltpu.make_async_copy(ostage.at[r], out_hbm.at[r], osems.at[c + i]) for i, r in enumerate(rows)]

    def b_out_last(c):
        ostage[cols(c), :] = b_proj(c).astype(bf16).T
        for cp in out_copies(c):
            cp.start()

    cp_wk.start()
    cp_x[0].start()
    xnT[pl.ds(D // 2, 8), :] = _pack(jnp.ones((16, S), f32))

    for first in (True, False):
        if first:
            cp_wk.wait()
            cp_x[1].start()
            transpose_w(wqa, K, wtA, K)
            cp_x[0].wait()
            cp_x[2].start()
            cp_x[3].start()
            load_x(0)
            cp_x[1].wait()
            load_x(1)
        a_k(0)
        if first:
            cp_x[2].wait()
            cp_x[3].wait()
            cp_wq.start()
            cp_wv.start()
            cp_woa.start()
            load_x(2)
            load_x(3)
        a_k(1)
        a_g(0)
        a_k(2)
        if first:
            cp_wq.wait()
            cp_wv.wait()
            cp_woa.wait()
            cp_wqb.start()
            cp_wob.start()
            transpose_w(wqa, Q, wtA, Q)
        a_g(1)
        a_k(3)
        a_g(2)
        a_q(0)
        a_g(3)
        if first:
            cp_wqb.wait()
            cp_wob.wait()
            transpose_w(wqb, K, wtB, K)
        a_q(1)
        kvs = a_kv()
        if first:
            transpose_w(wqb, Q, wtB, Q)
        a_q(2)
        a_m(kvs)
        a_den(0)
        a_den(1)
        a_den(2)
        if first:
            transpose_w(wqb, V, wtB, V)
        a_q(3)
        a_out(0)
        a_den(3)
        a_out(1)
        b_k(0)
        a_out(2)
        if first:
            transpose_w(wob, 0, wtB, O)
        b_q(0)
        b_k(1)
        a_out(3)
        b_q(1)
        b_k(2)
        b_k(3)
        b_q(2)
        b_q(3)
        for c in range(NC):
            b_v(c)
        attention(b_out_mid if first else b_out_last)
    for c in range(NC):
        for cp in out_copies(c):
            cp.wait()


def _call(x, wqa, woa, wqb, wob):
    vmem = pltpu.VMEM
    scratch = [
        vmem((S, D), bf16),
        vmem((D, 3 * D), bf16), vmem((D, D), bf16), vmem((D, 3 * D), bf16), vmem((D, D), bf16),
        vmem((S, D), bf16),
        pltpu.SemaphoreType.DMA((NC + 6,)), pltpu.SemaphoreType.DMA((NC + NT - 1,)),
        vmem((D, S), f32),
        vmem((D // 2 + 8, S), u32),
        vmem((D, D), u32),
        vmem((2 * D, D), u32),
        vmem((D // 2, S), u32),
        vmem((D + 16, D), f32),
        vmem((D // 2, D), u32),
        vmem((D // 2, D), u32),
        vmem((H, D), f32),
        vmem((D, S), f32),
        vmem((H, S), f32),
        vmem((D // 2, S), u32),
        vmem((D // 2, S), u32),
        vmem((D // 2, S), u32),
        vmem((NW, S // 2, 128), u32),
        vmem((D, S), f32),
        vmem((S, TC), f32), vmem((S, TC), f32),
    ]
    return pl.pallas_call(
        _kernel,
        out_shape=jax.ShapeDtypeStruct((S, D), bf16),
        in_specs=[pl.BlockSpec(memory_space=pl.ANY)] * 5,
        out_specs=pl.BlockSpec(memory_space=pl.ANY),
        scratch_shapes=scratch,
        compiler_params=pltpu.CompilerParams(vmem_limit_bytes=100 * 1024 * 1024),
        name="interleave",
    )(x, wqa, woa, wqb, wob)


@jax.jit
def pallas_interleave_layers__linear_attn_block__mha_block__prompt_kernel(
    A_x: jax.Array,
    A_wqkv: jax.Array,
    A_wo: jax.Array,
    B_x: jax.Array,
    B_wqkv: jax.Array,
    B_wo: jax.Array,
):
    del B_x
    out = _call(A_x.reshape(S, D), A_wqkv, A_wo, B_wqkv, B_wo)
    return out.reshape(A_x.shape)
```

```python
import jax
import jax.numpy as jnp
import numpy as np
from jax import lax
from jax.experimental import pallas as pl
from jax.experimental.pallas import tpu as pltpu

S = 2048
D = 640
H = 32
DH = D // H
TC = 512
NC = S // TC
NW = 6
CK = 128
HU = 4
SKEW = 2
DEP = 5
NT = 4
LN_EPS = 1e-5
PHI_EPS = 1e-6
QK_SCALE = float(DH ** -0.5 * np.log2(np.e))
ONES = np.uint32(0x3F803F80)

f32 = jnp.float32
bf16 = jnp.bfloat16
u32 = jnp.uint32
i32 = jnp.int32


def _pack(x):
    return pltpu.bitcast(x.astype(bf16), u32)


def _unpack(x):
    return pltpu.bitcast(x, bf16)


def _dot(a, b):
    return lax.dot_general(a, b, (((1,), (0,)), ((), ())), preferred_element_type=f32)


def _dot_nt(a, b):
    return lax.dot_general(a, b, (((1,), (1,)), ((), ())), preferred_element_type=f32)


def _phi(t):
    return jnp.where(t > 0, t + 1.0, jnp.exp(t)) + PHI_EPS


def _head_of(i):
    return (i * 3277) >> 16


def _band(j):
    h0, h1 = (128 * j) // DH, (128 * j + 127) // DH
    return (DH * h0) // 16 * 16, -(-(DH * (h1 + 1)) // 16) * 16


def _kernel(x_hbm, wqa_hbm, woa_hbm, wqb_hbm, wob_hbm, out_hbm,
            xraw, wqa, woa, wqb, wob, ostage, gT, mT, zsel, rden, gN, sems, osems,
            xT, xnT, wtA, wtB, pkT, pqo, pqs, qT, kT, kw, vT, sA, sB):
    Q, K, V, O = 0, D, 2 * D, 3 * D

    def cols(c):
        return pl.ds(c * TC, TC)

    def wrows(wt, r0, n=D):
        return _unpack(wt[pl.ds(r0 // 2, n // 2), :])

    def col_copy(src, dst, c0, s):
        return pltpu.make_async_copy(src.at[:, pl.ds(c0, D)], dst.at[:, pl.ds(c0, D)], sems.at[s])

    cp_x = [pltpu.make_async_copy(x_hbm.at[cols(c)], xraw.at[cols(c)], sems.at[c]) for c in range(NC)]
    cp_wk = col_copy(wqa_hbm, wqa, K, NC)
    cp_wq = col_copy(wqa_hbm, wqa, Q, NC + 1)
    cp_wv = col_copy(wqa_hbm, wqa, V, NC + 2)
    cp_woa = pltpu.make_async_copy(woa_hbm, woa, sems.at[NC + 3])
    cp_wqb = pltpu.make_async_copy(wqb_hbm, wqb, sems.at[NC + 4])
    cp_wob = pltpu.make_async_copy(wob_hbm, wob, sems.at[NC + 5])

    def transpose_w(src, c0, dst, r0):
        for j in range(0, D, 128):
            dst[pl.ds((r0 + j) // 2, 64), :] = pltpu.bitcast(src[:, pl.ds(c0 + j, 128)].T, u32)

    def layernorm(x, c):
        mean = jnp.sum(x, axis=0, keepdims=True) * (1.0 / D)
        xc = x - mean
        var = jnp.sum(xc * xc, axis=0, keepdims=True) * (1.0 / D)
        xnT[pl.ds(0, D // 2), cols(c)] = _pack(xc * lax.rsqrt(var + LN_EPS))

    def set_x(x, c):
        xT[:, cols(c)] = x
        layernorm(x, c)

    def load_x(c):
        set_x(xraw[cols(c), :].T.astype(f32), c)

    def proj(wt, r0, c):
        return _dot(wrows(wt, r0), _unpack(xnT[pl.ds(0, D // 2), cols(c)]))

    def scale_heads(c):
        low = lax.broadcasted_iota(i32, (8, TC), 0) < 4
        for g in range(H // 4):
            b = [jnp.broadcast_to(rden[pl.ds(4 * g + i, 1), cols(c)], (8, TC)) for i in range(4)]
            scale = jnp.concatenate(
                [b[0], b[0], jnp.where(low, b[0], b[1]), b[1], b[1],
                 b[2], b[2], jnp.where(low, b[2], b[3]), b[3], b[3]], axis=0)
            pqs[pl.ds(40 * g, 40), cols(c)] = _pack(pqo[pl.ds(80 * g, 80), cols(c)] * scale)

    def a_k(c):
        pkT[:, cols(c)] = _pack(_phi(proj(wtA, K, c)))

    def a_q(c):
        pqo[:, cols(c)] = _phi(proj(wtA, Q, c))

    def a_g(c):
        g = _dot_nt(_unpack(xnT[:, cols(c)]), _unpack(pkT[:, cols(c)]))
        gT[...] = g if c == 0 else gT[...] + g

    def a_kv():
        row = lax.broadcasted_iota(i32, (H, D), 0)
        col = lax.broadcasted_iota(i32, (H, D), 1)
        zsel[...] = jnp.where(_head_of(col) == row, jnp.broadcast_to(gT[pl.ds(D, 1), :], (H, D)), 0.0)
        for j in range(D // 128):
            gN[pl.ds(64 * j, 64), :] = pltpu.bitcast(
                gT[pl.ds(0, D), pl.ds(128 * j, 128)].astype(bf16).T, u32)
        out = []
        for j in range(D // 128):
            r0, r1 = _band(j)
            kv = _dot(wrows(gN, r0, r1 - r0), wqa[:, pl.ds(V + 128 * j, 128)])
            rr = lax.broadcasted_iota(i32, kv.shape, 0) + r0
            cc = lax.broadcasted_iota(i32, kv.shape, 1) + 128 * j
            out.append(jnp.where(_head_of(rr) == _head_of(cc), kv, 0.0).astype(bf16))
        return out

    def a_m(kvs):
        bands = [_band(j) for j in range(D // 128)]
        parts = [_dot(kv, woa[pl.ds(128 * j, 128), :]) for j, kv in enumerate(kvs)]
        for t in range(0, D, 128):
            cuts = sorted({t, t + 128} | {e for b in bands for e in b if t < e < t + 128})
            rows = []
            for lo, hi in zip(cuts[:-1], cuts[1:]):
                terms = [p[lo - r0:hi - r0] for p, (r0, r1) in zip(parts, bands) if r0 <= lo and hi <= r1]
                rows.append(sum(terms[1:], terms[0]))
            mT[:, pl.ds(t, 128)] = pltpu.bitcast(jnp.concatenate(rows, axis=0).astype(bf16).T, u32)

    def a_den(c):
        den = _dot(zsel[...], pqo[:, cols(c)].astype(bf16))
        rden[:, cols(c)] = 1.0 / (den + PHI_EPS)
        scale_heads(c)

    def a_out(c):
        set_x(xT[:, cols(c)] + _dot(wrows(mT, 0), _unpack(pqs[:, cols(c)])), c)

    def b_k(c):
        kT[:, cols(c)] = _pack(proj(wtB, K, c))
        for w in range(NW):
            r0 = min(60 * w - 4 * (w & 1), (D - 128) // 2)
            kt = _unpack(kT[pl.ds(r0, 64), cols(c)]).T
            kw[w, pl.ds(c * TC // 2, TC // 2), :] = pltpu.bitcast(kt, u32)

    def b_q(c):
        qT[:, cols(c)] = _pack(proj(wtB, Q, c) * QK_SCALE)

    def b_v(c):
        vT[:, cols(c)] = proj(wtB, V, c)

    def head_q(h, c):
        w = (h * 43) >> 8
        r0 = jnp.minimum(60 * w - 4 * (w & 1), (D - 128) // 2)
        lo = 10 * h - r0
        q = qT[pl.ds(pl.multiple_of(r0, 8), 64), cols(c)]
        i = lax.broadcasted_iota(i32, q.shape, 0)
        return w, _unpack(jnp.where((i >= lo) & (i < lo + 10), q, jnp.zeros_like(q)))

    def scores(w, q, dst, k, m):
        s = _dot(_unpack(kw[w, pl.ds(k * CK // 2, CK // 2), :]), q)
        dst[pl.ds(k * CK, CK), :] = s
        mm = jnp.max(s.reshape(CK // 8, 8, TC), axis=0)
        return mm if m is None else jnp.maximum(m, mm)

    def step(h, c, nxt, src, dst, m_cur, always, fill=()):
        n = S // CK
        off = 4 * (h & 1)
        ws = pl.multiple_of(DH * h - off, 8)

        def own(width):
            r = lax.broadcasted_iota(i32, (24, width), 0)
            return (r >= off) & (r < off + DH)

        own_ck = own(CK)
        hist, acc = [], []
        if nxt is not None:
            w, q = head_q(*nxt)

        def qk(k):
            hist.append(scores(w, q, dst, k, hist[-1] if hist else None))

        def pv(k):
            m = m_cur
            if len(hist) >= DEP:
                m = jnp.where(always, jnp.broadcast_to(m_cur, (8, TC)), hist[-DEP])
                m = jnp.broadcast_to(m[None], (CK // 8, 8, TC)).reshape(CK, TC)
            p = jnp.exp2(src[pl.ds(k * CK, CK), :] - m).astype(bf16)
            v = jnp.where(own_ck, vT[pl.ds(ws, 24), pl.ds(k * CK, CK)], 1.0)
            o = _dot(v, p)
            acc[:] = [o if not acc else acc[0] + o]

        events = [(k + SKEW + 0.5, k, pv) for k in range(n)] + list(fill)
        if nxt is not None:
            events += [(k + 0.0, k, qk) for k in range(n)]
        for _, k, fn in sorted(events, key=lambda e: e[0]):
            fn(k)
        o = acc[0]
        rden[pl.ds(h, 1), cols(c)] = jnp.where(off == 0, o[23:24, :], o[0:1, :])
        pqo[pl.ds(ws, 24), cols(c)] = jnp.where(own(TC), o, pqo[pl.ds(ws, 24), cols(c)])
        return None if nxt is None else jnp.max(hist[-1], axis=0, keepdims=True)

    def attention(b_out):
        w, q = head_q(jnp.int32(0), 0)
        m = None
        for k in range(S // CK):
            m = scores(w, q, sA, k, m)
        m = jnp.max(m, axis=0, keepdims=True)
        bufs = (sA, sB)

        def group(g, m, last=False):
            one = xnT[pl.ds(D // 2, 8), pl.ds(0, 128)]
            always = jnp.concatenate([one] * (TC // 128), axis=1) == ONES
            for j in range(HU):
                h = g * HU + j
                for c in range(NC):
                    nxt, fill = ((h, c + 1) if c + 1 < NC else (h + 1, 0)), ()
                    if last and j == HU - 1 and c == NC - 1:
                        nxt, fill = None, [(1.0 + 5 * i, i, b_out) for i in range(NC - 1)]
                    m = step(h, c, nxt, bufs[c % 2], bufs[(c + 1) % 2], m, always, fill)
            return m

        g, m = lax.fori_loop(0, H // HU - 1, lambda g, cr: (g + 1, group(g, cr[1])), (jnp.int32(0), m))
        group(g, m, last=True)
        b_out(NC - 1)

    def b_proj(c):
        rden[:, cols(c)] = 1.0 / rden[:, cols(c)]
        scale_heads(c)
        return xT[:, cols(c)] + _dot(wrows(wtB, O), _unpack(pqs[:, cols(c)]))

    def b_out_mid(c):
        set_x(b_proj(c), c)

    def out_copies(c):
        n = NT if c == NC - 1 else 1
        rows = [pl.ds(c * TC + i * (TC // n), TC // n) for i in range(n)]
        return [pltpu.make_async_copy(ostage.at[r], out_hbm.at[r], osems.at[c + i]) for i, r in enumerate(rows)]

    def b_out_last(c):
        ostage[cols(c), :] = b_proj(c).astype(bf16).T
        for cp in out_copies(c):
            cp.start()

    cp_wk.start()
    cp_x[0].start()
    xnT[pl.ds(D // 2, 8), :] = _pack(jnp.ones((16, S), f32))

    for first in (True, False):
        if first:
            cp_wk.wait()
            cp_x[1].start()
            transpose_w(wqa, K, wtA, K)
            cp_x[0].wait()
            cp_x[2].start()
            cp_x[3].start()
            load_x(0)
            cp_x[1].wait()
            load_x(1)
        a_k(0)
        if first:
            cp_x[2].wait()
            cp_x[3].wait()
            cp_wq.start()
            cp_wv.start()
            cp_woa.start()
            load_x(2)
            load_x(3)
        a_k(1)
        a_g(0)
        a_k(2)
        if first:
            cp_wq.wait()
            cp_wv.wait()
            cp_woa.wait()
            cp_wqb.start()
            cp_wob.start()
            transpose_w(wqa, Q, wtA, Q)
        a_g(1)
        a_k(3)
        a_g(2)
        a_q(0)
        a_g(3)
        if first:
            cp_wqb.wait()
            cp_wob.wait()
            transpose_w(wqb, K, wtB, K)
        a_q(1)
        kvs = a_kv()
        if first:
            transpose_w(wqb, Q, wtB, Q)
        a_den(0)
        a_q(2)
        a_m(kvs)
        a_den(1)
        if first:
            transpose_w(wqb, V, wtB, V)
        a_q(3)
        a_den(2)
        a_out(0)
        a_den(3)
        a_out(1)
        b_k(0)
        a_out(2)
        if first:
            transpose_w(wob, 0, wtB, O)
        b_q(0)
        b_k(1)
        a_out(3)
        b_q(1)
        b_k(2)
        b_k(3)
        b_q(2)
        b_q(3)
        for c in range(NC):
            b_v(c)
        attention(b_out_mid if first else b_out_last)
    for c in range(NC):
        for cp in out_copies(c):
            cp.wait()


def _call(x, wqa, woa, wqb, wob):
    vmem = pltpu.VMEM
    scratch = [
        vmem((S, D), bf16),
        vmem((D, 3 * D), bf16), vmem((D, D), bf16), vmem((D, 3 * D), bf16), vmem((D, D), bf16),
        vmem((S, D), bf16),
        vmem((D + 16, D), f32),
        vmem((D // 2, D), u32),
        vmem((H, D), f32),
        vmem((H, S), f32),
        vmem((D // 2, D), u32),
        pltpu.SemaphoreType.DMA((NC + 6,)),
        pltpu.SemaphoreType.DMA((NC + NT - 1,)),
        vmem((D, S), f32),
        vmem((D // 2 + 8, S), u32),
        vmem((D, D), u32),
        vmem((2 * D, D), u32),
        vmem((D // 2, S), u32),
        vmem((D, S), f32),
        vmem((D // 2, S), u32),
        vmem((D // 2, S), u32),
        vmem((D // 2, S), u32),
        vmem((NW, S // 2, 128), u32),
        vmem((D, S), f32),
        vmem((S, TC), f32), vmem((S, TC), f32),
    ]
    return pl.pallas_call(
        _kernel,
        out_shape=jax.ShapeDtypeStruct((S, D), bf16),
        in_specs=[pl.BlockSpec(memory_space=pl.ANY)] * 5,
        out_specs=pl.BlockSpec(memory_space=pl.ANY),
        scratch_shapes=scratch,
        compiler_params=pltpu.CompilerParams(vmem_limit_bytes=100 * 1024 * 1024),
        name="interleave",
    )(x, wqa, woa, wqb, wob)


@jax.jit
def pallas_interleave_layers__linear_attn_block__mha_block__prompt_kernel(
    A_x: jax.Array,
    A_wqkv: jax.Array,
    A_wo: jax.Array,
    B_x: jax.Array,
    B_wqkv: jax.Array,
    B_wo: jax.Array,
):
    del B_x
    out = _call(A_x.reshape(S, D), A_wqkv, A_wo, B_wqkv, B_wo)
    return out.reshape(A_x.shape)
```
